```python
import os as _os
_os.environ.setdefault("JAX_PLATFORMS", "cpu")
import jax
import jax.numpy as jnp

def _softmax(x, axis=-1):
    return jax.nn.softmax(x, axis=axis)
def _gelu(x):
    return jax.nn.gelu(x, approximate=True)
def _silu(x):
    return jax.nn.silu(x)
def _sigmoid(x):
    return jax.nn.sigmoid(x)
def _layernorm(x, axis=-1, eps=1e-5):
    m = jnp.mean(x, axis=axis, keepdims=True)
    v = jnp.var(x, axis=axis, keepdims=True)
    return (x - m) / jnp.sqrt(v + eps)
def _scatter_add(tgt, idx, src, axis=0):
    return tgt.at[idx].add(src)
def _segment_sum(src, seg, n):
    return jax.ops.segment_sum(src, seg, n)
class _Rng:
    def __init__(self, key):
        self._k = key
    def _next(self):
        self._k, sub = jax.random.split(self._k)
        return sub
    def normal(self, shape):
        return jax.random.normal(self._next(), shape, dtype=jnp.bfloat16)
    def randint(self, lo, hi, shape):
        return jax.random.randint(self._next(), shape, lo, hi, dtype=jnp.int32)
    def uniform(self, shape, lo=0.0, hi=1.0):
        return jax.random.uniform(self._next(), shape, jnp.bfloat16, lo, hi)
    def permutation(self, n):
        return jax.random.permutation(self._next(), n)


kernel_name = 'standalone__cross_network_dcn_v2__recsys'

def setup_inputs():
    _rng = _Rng(jax.random.key(int.from_bytes(__import__("os").urandom(4), "little")))
    _w = (lambda a: (lambda t: t.astype(jnp.bfloat16) if jnp.issubdtype(t.dtype, jnp.floating) else t)(jnp.asarray(a)))
    B, F, D, L = 16384, 26, 16, 6
    Din = min(F * D, 512)
    R = max(Din // 4, 2)
    sc = Din ** -0.5
    return {
        "x0": _w((lambda *s: _rng.normal(s) * 0.05)(B, Din)),
        "U":  _w((lambda *s: _rng.normal(s) * 1.6)(L, Din, R) * sc),
        "V":  _w((lambda *s: _rng.normal(s) * 1.6)(L, R, Din) * sc),
        "bs": _w((lambda *s: _rng.normal(s) * 0.05)(L, Din)),
    }

def reference(x0, U, V, bs):
    x = x0
    for l in range(U.shape[0]):
        h = jnp.einsum('rd,bd->br', V[l], x)
        h = jnp.einsum('dr,br->bd', U[l], h)
        x = x0 * (h + bs[l]) + x
    return x
```

```python
import jax
import jax.numpy as jnp
from jax import lax
import jax.experimental.pallas as pl
import jax.experimental.pallas.tpu as pltpu

F32, BF16, U32 = jnp.float32, jnp.bfloat16, jnp.uint32
LANES = 128
TW = 512
NT = 2
G = 3


def _mm(a, b):
    return lax.dot_general(a, b, (((1,), (0,)), ((), ())), preferred_element_type=F32)


def _kernel(x_hbm, u_hbm, v_hbm, b_hbm, o_hbm,
            xin, xout, u_ref, v_ref, b_ref, vf_ref, ua_ref, vb_ref, bb_ref, xt_ref,
            in_sem, out_sem, w_sem):
    L, D, R = u_ref.shape
    KP = D // LANES * LANES
    NLO = D - KP - (LANES - R)
    CW = TW * NT
    n_chunks = x_hbm.shape[1] // CW
    n_it = (n_chunks - 1) // G

    def in_copies(it):
        return [pltpu.make_async_copy(
            x_hbm.at[:, pl.ds(pl.multiple_of((1 + it * G + g) * CW, CW), CW)],
            xin.at[1 + it * G + g], in_sem.at[it % 2]) for g in range(G)]

    cp = {}
    for l in range(L):
        cp[f"V{l}"] = pltpu.make_async_copy(v_hbm.at[l], v_ref.at[l], w_sem.at[2 * l])
        cp[f"U{l}"] = pltpu.make_async_copy(u_hbm.at[l], u_ref.at[l], w_sem.at[2 * l + 1])
    cp["b"] = pltpu.make_async_copy(b_hbm, b_ref, w_sem.at[2 * L])
    cp["xA"] = pltpu.make_async_copy(x_hbm.at[:, pl.ds(0, TW)], xin.at[0, :, pl.ds(0, TW)], w_sem.at[2 * L + 1])
    cp["xB"] = pltpu.make_async_copy(x_hbm.at[:, pl.ds(TW, TW)], xin.at[0, :, pl.ds(TW, TW)], w_sem.at[2 * L + 2])

    def build(l):
        lane = lax.broadcasted_iota(jnp.int32, (R, LANES), 1)
        row = lax.broadcasted_iota(jnp.int32, (R, LANES), 0)
        v = v_ref[l].astype(F32)
        vf_ref[l] = v[:, :KP]
        vt = jnp.concatenate([v[:, KP:], jnp.zeros((R, LANES - (D - KP)), F32)], axis=1)
        for a in range(NLO):
            vb_ref[l, a] = jnp.broadcast_to(vt[:, a:a + 1], (R, LANES))
        vr = pltpu.roll(vt, LANES - (D - KP), axis=1)
        vp = jnp.where(lane < R, (lane == row).astype(F32), vr).astype(BF16)
        ua_ref[l] = pltpu.bitcast(_mm(u_ref[l], vp).astype(BF16), U32)
        brow = jnp.concatenate([b_ref[...].astype(F32)[l:l + 1], jnp.zeros((1, KP + LANES - D), F32)], axis=1)
        bb_ref[l] = jnp.broadcast_to(brow, (LANES, KP + LANES)).T[:D]

    def tile_cols(x):
        return jnp.concatenate([x] * (TW // LANES), axis=1)

    def group(c, ops):
        st = {}

        def cols(t):
            return slice(t * TW, (t + 1) * TW)

        def p1(t, l):
            if l == 0:
                xt_ref[t] = xin[c, KP:D, cols(t)].astype(F32)
                xb = xin[c, :KP, cols(t)]
            else:
                xb = pltpu.bitcast(st["xw", t][:KP // 2], BF16)
            xt = xt_ref[t]
            h = None
            for a in range(NLO):
                p = tile_cols(vb_ref[l, a]) * xt[a:a + 1, :]
                h = p if h is None else h + p
            h = h + _mm(vf_ref[l], xb)
            st["hb", t] = jnp.concatenate([h, xt[NLO:]], axis=0).astype(BF16)

        def p2(t, l):
            g = _mm(pltpu.bitcast(ua_ref[l], BF16), st["hb", t]) + tile_cols(bb_ref[l])
            x0 = xin[c, :, cols(t)].astype(F32)
            xp = x0 if l == 0 else pltpu.bitcast(st["xw", t], BF16).astype(F32)
            xn = x0 * g + xp
            if l == L - 1:
                for r0, r1 in ((0, D // 2), (D // 2, D)):
                    xout[c, r0:r1, cols(t)] = xn[r0:r1].astype(BF16)
                    pltpu.make_async_copy(
                        xout.at[c, r0:r1, cols(t)],
                        o_hbm.at[r0:r1, pl.ds(pl.multiple_of(c * CW + t * TW, TW), TW)], out_sem).start()
            else:
                st["xw", t] = pltpu.bitcast(xn.astype(BF16), U32)
                xt_ref[t] = xn[KP:]

        for op in ops:
            k = op.split(":")
            if k[0] == "p1":
                p1(int(k[1]), int(k[2]))
            elif k[0] == "p2":
                p2(int(k[1]), int(k[2]))
            elif k[0] == "B":
                build(int(k[1]))
            elif op == "s:next":
                for d in in_copies(0):
                    d.start()
            elif k[0] == "s":
                cp[k[1]].start()
            else:
                cp[k[1]].wait()

    first = ('s:V0 s:U0 s:b s:V1 s:U1 s:xA w:V0 w:U0 w:b s:xB B:0 w:V1 w:U1 '
             's:V2 s:U2 s:V3 s:U3 s:V4 s:U4 s:V5 s:U5 B:1 w:xA '
             'p1:0:0 p2:0:0 w:xB s:next p1:1:0 p1:0:1 p2:1:0 p2:0:1 p1:1:1 '
             'w:V2 w:U2 w:V3 w:U3 w:V4 w:U4 w:V5 w:U5 '
             'B:2 p2:1:1 p1:0:2 B:3 p1:1:2 p2:0:2 p2:1:2 p1:0:3 B:4 p1:1:3 p2:0:3 p2:1:3 '
             'p1:0:4 B:5 p1:1:4 p2:0:4 p2:1:4 p1:0:5 p1:1:5 p2:0:5 p2:1:5').split()
    steady = [f"p{p}:{t}:{l}" for l in range(L) for p in (1, 2) for t in range(NT)]
    group(0, first)

    def body(it, carry):
        @pl.when(it + 1 < n_it)
        def _():
            for d in in_copies(it + 1):
                d.start()
        for d in in_copies(it):
            d.wait()
        for g in range(G):
            group(1 + it * G + g, steady)
        return carry

    lax.fori_loop(0, n_it, body, 0)
    pltpu.make_async_copy(xout, xout, out_sem).wait()


@jax.jit
def pallas_standalone__cross_network_dcn_v2__recsys_kernel(x0, U, V, bs):
    B, D = x0.shape
    L, _, R = U.shape
    CW = TW * NT
    n_chunks = B // CW
    KP = D // LANES * LANES
    NLO = D - KP - (LANES - R)
    any_spec = pl.BlockSpec(memory_space=pl.ANY)
    out = pl.pallas_call(
        _kernel,
        in_specs=[any_spec] * 4,
        out_specs=any_spec,
        out_shape=jax.ShapeDtypeStruct((D, B), x0.dtype),
        scratch_shapes=[
            pltpu.VMEM((n_chunks, D, CW), BF16), pltpu.VMEM((n_chunks, D, CW), BF16),
            pltpu.VMEM((L, D, R), BF16), pltpu.VMEM((L, R, D), BF16), pltpu.VMEM((L, D), BF16),
            pltpu.VMEM((L, R, KP), F32), pltpu.VMEM((L, D // 2, LANES), U32),
            pltpu.VMEM((L, NLO, R, LANES), F32), pltpu.VMEM((L, D, LANES), F32),
            pltpu.VMEM((NT, D - KP, TW), F32),
            pltpu.SemaphoreType.DMA((2,)), pltpu.SemaphoreType.DMA(()),
            pltpu.SemaphoreType.DMA((2 * L + 3,)),
        ],
        compiler_params=pltpu.CompilerParams(
            vmem_limit_bytes=110 * 1024 * 1024,
            flags={"XLA_TPU_EVENLY_DISTRIBUTE_CRITICAL_NODES": True}),
    )(x0.T, U, V, bs)
    return out.T
```

```python
import functools

import jax
import jax.numpy as jnp
from jax import lax
import jax.experimental.pallas as pl
import jax.experimental.pallas.tpu as pltpu

F32, BF16, U32 = jnp.float32, jnp.bfloat16, jnp.uint32
LANES = 128
TILE = 256
WINDOW = 6
LAG = 3
HEAD = 512
BODY_TILES = 18


def _mm(a, b):
    return lax.dot_general(a, b, (((1,), (0,)), ((), ())), preferred_element_type=F32)


def _mm_nt(a, b):
    return lax.dot_general(a, b, (((1,), (1,)), ((), ())), preferred_element_type=F32)


def _pad_to(x, rows, cols):
    if x.shape[1] < cols:
        x = jnp.concatenate([x, jnp.zeros((x.shape[0], cols - x.shape[1]), F32)], axis=1)
    if x.shape[0] < rows:
        x = jnp.concatenate([x, jnp.zeros((rows - x.shape[0], cols), F32)], axis=0)
    return x


def _rolling(tiles, n_layers):
    units = [(t, l)
             for g in range(0, len(tiles), WINDOW)
             for l in range(n_layers)
             for t in tiles[g:g + WINDOW]]
    order = []
    for i in range(len(units) + LAG):
        if i < len(units):
            order.append((1,) + units[i])
        if i >= LAG:
            order.append((2,) + units[i - LAG])
    return order


def _split(d, r):
    km = d // LANES * LANES
    return km, d - km - (LANES - r - 1)


def _kernel(x_hbm, u_hbm, v_hbm, b_hbm, o_hbm,
            xin_head, xin_body, xout_head, xout_body, u_raw, v_raw, b_raw,
            vm_ref, vv_ref, ua_ref, xm_ref, xt_ref,
            head_sem, in_sem, out_sem):
    n_layers, d, r = u_raw.shape
    km, nv = _split(d, r)
    d_pad = km + LANES
    head_cols = xin_head.shape[1]
    n_iter, _, body_cols = xin_body.shape

    def v_tail(l):
        return _pad_to(v_raw[l, :, km:].astype(F32), r, LANES)

    def build_v(l):
        vm_ref[l] = v_raw[l, :, :km].astype(F32)
        vt = v_tail(l)
        for a in range(nv):
            vv_ref[l, a] = jnp.broadcast_to(vt[:, a:a + 1], (r, LANES))

    def build_u(l):
        bias = _pad_to(b_raw[...].astype(F32)[l:l + 1], 1, d_pad)
        vt_t = _pad_to(v_tail(l), LANES, LANES).T
        w_t = _pad_to(_mm_nt(vt_t[nv - 1:d - km, :r], u_raw[l]), LANES - r, d_pad)
        first = lax.broadcasted_iota(jnp.int32, (8, d_pad), 0) == 0
        extra = jnp.concatenate(
            [jnp.zeros((r, d_pad), F32), jnp.where(first, bias, w_t[:8]), w_t[8:]], axis=0)
        ua = _pad_to(u_raw[l].astype(F32), d, LANES) + extra.T[:d]
        ua_ref[l] = pltpu.bitcast(ua.astype(BF16), U32)

    def phases(x_in, x_out, col0, widths, sem):
        starts = [sum(widths[:t]) for t in range(len(widths))]
        h_aug = {}

        def phase1(t, l):
            cols = slice(starts[t], starts[t] + widths[t])
            if l == 0:
                xt_ref[:, cols] = x_in[km:d, cols].astype(F32)
                xm = x_in[:km, cols]
            else:
                xm = xm_ref[:, cols].astype(BF16)
            xt = xt_ref[:, cols]
            terms = [jnp.concatenate([vv_ref[l, a]] * (widths[t] // LANES), axis=1) * xt[a:a + 1]
                     for a in range(nv)]
            h = functools.reduce(lambda p, q: p + q, terms) + _mm(vm_ref[l], xm)
            xw = xt[nv - 1:]
            xw = jnp.where(lax.broadcasted_iota(jnp.int32, xw.shape, 0) == 0, 1.0, xw)
            h_aug[t] = jnp.concatenate([h, xw], axis=0).astype(BF16)

        def phase2(t, l):
            cols = slice(starts[t], starts[t] + widths[t])
            g = _mm(pltpu.bitcast(ua_ref[l], BF16), h_aug.pop(t))
            x0 = x_in[:, cols].astype(F32)
            x = x0 if l == 0 else jnp.concatenate([xm_ref[:, cols], xt_ref[:, cols]], axis=0)
            x = x0 * g + x
            if l < n_layers - 1:
                xm_ref[:, cols] = x[:km]
                xt_ref[:, cols] = x[km:]
                return
            dst_cols = pl.ds(pl.multiple_of(col0 + starts[t], LANES), widths[t])
            for rows in (slice(0, d // 2), slice(d // 2, d)):
                x_out[rows, cols] = x[rows].astype(x_out.dtype)
                pltpu.make_async_copy(x_out.at[rows, cols], o_hbm.at[rows, dst_cols], sem).start()

        def run(order):
            for phase, t, l in order:
                (phase1 if phase == 1 else phase2)(t, l)

        return run

    def head_cols_copy(lo, hi):
        return x_hbm.at[:, lo:hi], xin_head.at[:, lo:hi]

    groups = [
        [(v_hbm.at[0], v_raw.at[0]), (u_hbm.at[0], u_raw.at[0]), (b_hbm, b_raw)],
        [head_cols_copy(0, HEAD)],
        [(v_hbm.at[1], v_raw.at[1]), (u_hbm.at[1], u_raw.at[1]), head_cols_copy(HEAD, 2 * HEAD)],
        [(v_hbm.at[2:], v_raw.at[2:]), (u_hbm.at[2:], u_raw.at[2:])],
        [head_cols_copy(2 * HEAD, head_cols)],
    ]
    groups = [[pltpu.make_async_copy(src, dst, head_sem.at[i]) for src, dst in group]
              for i, group in enumerate(groups)]

    def start(i):
        for copy in groups[i]:
            copy.start()

    def wait(i):
        for copy in groups[i]:
            copy.wait()

    def body_copy(it):
        cols = pl.ds(pl.multiple_of(head_cols + it * body_cols, LANES), body_cols)
        return pltpu.make_async_copy(x_hbm.at[:, cols], xin_body.at[it], in_sem.at[it])

    widths = [HEAD, HEAD] + [TILE] * WINDOW
    run = phases(xin_head, xout_head, 0, widths, out_sem.at[0])
    start(0)
    start(1)
    wait(0)
    start(2)
    build_v(0)
    build_u(0)
    wait(1)
    start(3)
    run([(1, 0, 0), (2, 0, 0)])
    wait(2)
    start(4)
    for it in range(n_iter):
        body_copy(it).start(priority=1)
    run([(1, 1, 0)])
    build_v(1)
    run([(1, 0, 1)])
    build_u(1)
    run([(2, 1, 0), (2, 0, 1), (1, 1, 1)])
    wait(3)
    build_v(2)
    run([(2, 1, 1)])
    for l in range(2, n_layers):
        run([(1, 0, l)])
        build_u(l)
        run([(1, 1, l)])
        if l + 1 < n_layers:
            build_v(l + 1)
        run([(2, 0, l), (2, 1, l)])
    wait(4)
    run(_rolling(list(range(2, len(widths))), n_layers))

    def body(it, carry):
        body_copy(it).wait()
        run = phases(xin_body.at[it], xout_body.at[it], head_cols + it * body_cols,
                     [TILE] * BODY_TILES, out_sem.at[1])
        run(_rolling(list(range(BODY_TILES)), n_layers))
        return carry

    lax.fori_loop(0, n_iter, body, 0)

    pltpu.make_async_copy(xout_head, xout_head, out_sem.at[0]).wait()
    pltpu.make_async_copy(xout_body, xout_body, out_sem.at[1]).wait()


@jax.jit
def pallas_standalone__cross_network_dcn_v2__recsys_kernel(
    x0: jax.Array,
    U: jax.Array,
    V: jax.Array,
    bs: jax.Array,
):
    batch, d = x0.shape
    n_layers, _, r = U.shape
    km, nv = _split(d, r)
    head_cols = 2 * HEAD + WINDOW * TILE
    body_cols = BODY_TILES * TILE
    n_iter = (batch - head_cols) // body_cols
    assert head_cols + n_iter * body_cols == batch and n_layers >= 3
    assert r % 8 == 0 and d % 32 == 0 and nv % 8 == 1

    hbm = pl.BlockSpec(memory_space=pl.ANY)
    out_t = pl.pallas_call(
        _kernel,
        in_specs=[hbm] * 4,
        out_specs=hbm,
        out_shape=jax.ShapeDtypeStruct((d, batch), x0.dtype),
        scratch_shapes=[
            pltpu.VMEM((d, head_cols), x0.dtype),
            pltpu.VMEM((n_iter, d, body_cols), x0.dtype),
            pltpu.VMEM((d, head_cols), x0.dtype),
            pltpu.VMEM((n_iter, d, body_cols), x0.dtype),
            pltpu.VMEM(U.shape, U.dtype),
            pltpu.VMEM(V.shape, V.dtype),
            pltpu.VMEM(bs.shape, bs.dtype),
            pltpu.VMEM((n_layers, r, km), F32),
            pltpu.VMEM((n_layers, nv, r, LANES), F32),
            pltpu.VMEM((n_layers, d // 2, LANES), U32),
            pltpu.VMEM((km, body_cols), F32),
            pltpu.VMEM((d - km, body_cols), F32),
            pltpu.SemaphoreType.DMA((5,)),
            pltpu.SemaphoreType.DMA((n_iter,)),
            pltpu.SemaphoreType.DMA((2,)),
        ],
        compiler_params=pltpu.CompilerParams(
            vmem_limit_bytes=100 * 1024 * 1024,
            flags={"XLA_TPU_EVENLY_DISTRIBUTE_CRITICAL_NODES": True},
        ),
    )(x0.T, U, V, bs)
    return out_t.T
```

```python
import functools

import jax
import jax.numpy as jnp
from jax import lax
import jax.experimental.pallas as pl
import jax.experimental.pallas.tpu as pltpu

F32, BF16, U32 = jnp.float32, jnp.bfloat16, jnp.uint32
LANES = 128
TILE = 256
WINDOW = 6
LAG = 3
HEAD = 512
BODY_TILES = 18
SLIVER = 48


def _mm(a, b):
    return lax.dot_general(a, b, (((1,), (0,)), ((), ())), preferred_element_type=F32)


def _mm_nt(a, b):
    return lax.dot_general(a, b, (((1,), (1,)), ((), ())), preferred_element_type=F32)


def _pad_to(x, rows, cols):
    if x.shape[1] < cols:
        x = jnp.concatenate([x, jnp.zeros((x.shape[0], cols - x.shape[1]), F32)], axis=1)
    if x.shape[0] < rows:
        x = jnp.concatenate([x, jnp.zeros((rows - x.shape[0], cols), F32)], axis=0)
    return x


def _rolling(tiles, n_layers, taper=False):
    units = [(t, l)
             for g in range(0, len(tiles), WINDOW)
             for l in range(n_layers)
             for t in tiles[g:g + WINDOW]]
    order, done = [], 0
    for i, unit in enumerate(units):
        order.append((1,) + unit)
        lag = 1 if taper and i >= len(units) - WINDOW - LAG else LAG
        while done <= i - lag:
            order.append((2,) + units[done])
            done += 1
    order += [(2,) + unit for unit in units[done:]]
    if taper:
        order[-2:-1] = [order[-2] + (0, SLIVER), order[-2] + (SLIVER, None)]
    return order


def _split(d, r):
    km = d // LANES * LANES
    return km, d - km - (LANES - r - 1)


def _kernel(x_hbm, u_hbm, v_hbm, b_hbm, o_hbm,
            xin_head, xin_body, xout_head, xout_body, u_raw, v_raw, b_raw,
            vm_ref, vv_ref, ua_ref, xm_ref, xt_ref,
            head_sem, in_sem, out_sem):
    n_layers, d, r = u_raw.shape
    km, nv = _split(d, r)
    d_pad = km + LANES
    head_cols = xin_head.shape[1]
    n_iter, _, body_cols = xin_body.shape

    def v_tail(l):
        return _pad_to(v_raw[l, :, km:].astype(F32), r, LANES)

    def build_v(l):
        vm_ref[l] = v_raw[l, :, :km].astype(F32)
        vt = v_tail(l)
        for a in range(nv):
            vv_ref[l, a] = jnp.broadcast_to(vt[:, a:a + 1], (r, LANES))

    def build_u(l):
        bias = _pad_to(b_raw[...].astype(F32)[l:l + 1], 1, d_pad)
        vt_t = _pad_to(v_tail(l), LANES, LANES).T
        w_t = _pad_to(_mm_nt(vt_t[nv - 1:d - km, :r], u_raw[l]), LANES - r, d_pad)
        first = lax.broadcasted_iota(jnp.int32, (8, d_pad), 0) == 0
        extra = jnp.concatenate(
            [jnp.zeros((r, d_pad), F32), jnp.where(first, bias, w_t[:8]), w_t[8:]], axis=0)
        ua = _pad_to(u_raw[l].astype(F32), d, LANES) + extra.T[:d]
        ua_ref[l] = pltpu.bitcast(ua.astype(BF16), U32)

    def phases(x_in, x_out, col0, widths, sem):
        starts = [sum(widths[:t]) for t in range(len(widths))]
        h_aug = {}

        def phase1(t, l):
            cols = slice(starts[t], starts[t] + widths[t])
            if l == 0:
                xt_ref[:, cols] = x_in[km:d, cols].astype(F32)
                xm = x_in[:km, cols]
            else:
                xm = xm_ref[:, cols].astype(BF16)
            xt = xt_ref[:, cols]
            terms = [jnp.concatenate([vv_ref[l, a]] * (widths[t] // LANES), axis=1) * xt[a:a + 1]
                     for a in range(nv)]
            h = functools.reduce(lambda p, q: p + q, terms) + _mm(vm_ref[l], xm)
            xw = xt[nv - 1:]
            xw = jnp.where(lax.broadcasted_iota(jnp.int32, xw.shape, 0) == 0, 1.0, xw)
            h_aug[t] = jnp.concatenate([h, xw], axis=0).astype(BF16)

        def phase2(t, l, lo=0, hi=None):
            hi = d if hi is None else hi
            cols = slice(starts[t], starts[t] + widths[t])
            g = _mm(pltpu.bitcast(ua_ref[l, lo // 2:hi // 2], BF16), h_aug[t])
            x0 = x_in[lo:hi, cols].astype(F32)
            if l == 0:
                x = x0
            elif hi <= km:
                x = xm_ref[lo:hi, cols]
            else:
                x = jnp.concatenate([xm_ref[lo:km, cols], xt_ref[:, cols]], axis=0)
            x = x0 * g + x
            if l < n_layers - 1:
                xm_ref[:, cols] = x[:km]
                xt_ref[:, cols] = x[km:]
                return
            dst_cols = pl.ds(pl.multiple_of(col0 + starts[t], LANES), widths[t])
            for r0, r1 in ((lo, min(hi, d // 2)), (max(lo, d // 2), hi)):
                if r0 < r1:
                    x_out[r0:r1, cols] = x[r0 - lo:r1 - lo].astype(x_out.dtype)
                    pltpu.make_async_copy(
                        x_out.at[r0:r1, cols], o_hbm.at[r0:r1, dst_cols], sem).start()

        def run(order):
            for phase, *args in order:
                (phase1 if phase == 1 else phase2)(*args)

        return run

    def head_cols_copy(lo, hi):
        return x_hbm.at[:, lo:hi], xin_head.at[:, lo:hi]

    groups = [
        [(v_hbm.at[0], v_raw.at[0]), (u_hbm.at[0], u_raw.at[0]), (b_hbm, b_raw)],
        [head_cols_copy(0, HEAD)],
        [(v_hbm.at[1], v_raw.at[1]), (u_hbm.at[1], u_raw.at[1]), head_cols_copy(HEAD, 2 * HEAD)],
        [(v_hbm.at[2:], v_raw.at[2:]), (u_hbm.at[2:], u_raw.at[2:])],
        [head_cols_copy(2 * HEAD, head_cols)],
    ]
    groups = [[pltpu.make_async_copy(src, dst, head_sem.at[i]) for src, dst in group]
              for i, group in enumerate(groups)]

    def start(i):
        for copy in groups[i]:
            copy.start()

    def wait(i):
        for copy in groups[i]:
            copy.wait()

    def body_copy(it):
        cols = pl.ds(pl.multiple_of(head_cols + it * body_cols, LANES), body_cols)
        return pltpu.make_async_copy(x_hbm.at[:, cols], xin_body.at[it], in_sem.at[it])

    widths = [HEAD, HEAD] + [TILE] * WINDOW
    run = phases(xin_head, xout_head, 0, widths, out_sem.at[0])
    start(0)
    start(1)
    wait(0)
    start(2)
    build_v(0)
    build_u(0)
    wait(1)
    start(3)
    run([(1, 0, 0), (2, 0, 0)])
    wait(2)
    start(4)
    for it in range(n_iter):
        body_copy(it).start(priority=1)
    run([(1, 1, 0)])
    build_v(1)
    run([(1, 0, 1)])
    build_u(1)
    run([(2, 1, 0), (2, 0, 1), (1, 1, 1)])
    wait(3)
    build_v(2)
    run([(2, 1, 1)])
    for l in range(2, n_layers):
        run([(1, 0, l)])
        build_u(l)
        run([(1, 1, l)])
        if l + 1 < n_layers:
            build_v(l + 1)
        run([(2, 0, l), (2, 1, l)])
    wait(4)
    run(_rolling(list(range(2, len(widths))), n_layers))

    def body(it, carry):
        body_copy(it).wait()
        run = phases(xin_body.at[it], xout_body.at[it], head_cols + it * body_cols,
                     [TILE] * BODY_TILES, out_sem.at[1])
        run(_rolling(list(range(BODY_TILES)), n_layers, taper=True))
        return carry

    lax.fori_loop(0, n_iter, body, 0)

    pltpu.make_async_copy(xout_head, xout_head, out_sem.at[0]).wait()
    pltpu.make_async_copy(xout_body, xout_body, out_sem.at[1]).wait()


@jax.jit
def pallas_standalone__cross_network_dcn_v2__recsys_kernel(
    x0: jax.Array,
    U: jax.Array,
    V: jax.Array,
    bs: jax.Array,
):
    batch, d = x0.shape
    n_layers, _, r = U.shape
    km, nv = _split(d, r)
    head_cols = 2 * HEAD + WINDOW * TILE
    body_cols = BODY_TILES * TILE
    n_iter = (batch - head_cols) // body_cols
    assert head_cols + n_iter * body_cols == batch and n_layers >= 3
    assert r % 8 == 0 and d % 32 == 0 and nv % 8 == 1

    hbm = pl.BlockSpec(memory_space=pl.ANY)
    out_t = pl.pallas_call(
        _kernel,
        in_specs=[hbm] * 4,
        out_specs=hbm,
        out_shape=jax.ShapeDtypeStruct((d, batch), x0.dtype),
        scratch_shapes=[
            pltpu.VMEM((d, head_cols), x0.dtype),
            pltpu.VMEM((n_iter, d, body_cols), x0.dtype),
            pltpu.VMEM((d, head_cols), x0.dtype),
            pltpu.VMEM((n_iter, d, body_cols), x0.dtype),
            pltpu.VMEM(U.shape, U.dtype),
            pltpu.VMEM(V.shape, V.dtype),
            pltpu.VMEM(bs.shape, bs.dtype),
            pltpu.VMEM((n_layers, r, km), F32),
            pltpu.VMEM((n_layers, nv, r, LANES), F32),
            pltpu.VMEM((n_layers, d // 2, LANES), U32),
            pltpu.VMEM((km, body_cols), F32),
            pltpu.VMEM((d - km, body_cols), F32),
            pltpu.SemaphoreType.DMA((5,)),
            pltpu.SemaphoreType.DMA((n_iter,)),
            pltpu.SemaphoreType.DMA((2,)),
        ],
        compiler_params=pltpu.CompilerParams(vmem_limit_bytes=100 * 1024 * 1024),
    )(x0.T, U, V, bs)
    return out_t.T
```
